```python
import jax
import jax.numpy as jnp

def _softmax(x, axis=-1):
    return jax.nn.softmax(x, axis=axis)
def _gelu(x):
    return jax.nn.gelu(x, approximate=True)
def _silu(x):
    return jax.nn.silu(x)
def _sigmoid(x):
    return jax.nn.sigmoid(x)
def _layernorm(x, axis=-1, eps=1e-5):
    m = jnp.mean(x, axis=axis, keepdims=True)
    v = jnp.var(x, axis=axis, keepdims=True)
    return (x - m) / jnp.sqrt(v + eps)
def _scatter_add(tgt, idx, src, axis=0):
    return tgt.at[idx].add(src)
def _segment_sum(src, seg, n):
    return jax.ops.segment_sum(src, seg, n)
class _Rng:
    def __init__(self, key):
        self._k = key
    def _next(self):
        self._k, sub = jax.random.split(self._k)
        return sub
    def normal(self, shape):
        return jax.random.normal(self._next(), shape, dtype=jnp.bfloat16)
    def randint(self, lo, hi, shape):
        return jax.random.randint(self._next(), shape, lo, hi, dtype=jnp.int32)
    def uniform(self, shape, lo=0.0, hi=1.0):
        return jax.random.uniform(self._next(), shape, jnp.bfloat16, lo, hi)
    def permutation(self, n):
        return jax.random.permutation(self._next(), n)


kernel_name = 'standalone__dcn_v2_cross__recsys'

def setup_inputs():
    _rng = _Rng(jax.random.key(int.from_bytes(__import__("os").urandom(4), "little")))
    _w = (lambda a: (lambda t: t.astype(jnp.bfloat16) if jnp.issubdtype(t.dtype, jnp.floating) else t)(jnp.asarray(a)))
    B, F, D, L = 16384, 26, 128, 6
    Din = min(F * D, 1024)
    return {
        "x0": _w((lambda *s: _rng.normal(s) * 0.05)(B, Din)),
        "ws": _w((lambda *s: _rng.normal(s) * 0.05)(L, Din, Din)),
        "bs": _w((lambda *s: _rng.normal(s) * 0.05)(L, Din)),
    }

def reference(x0, ws, bs):
    x = x0
    for l in range(ws.shape[0]):
        x = x0 * (x @ ws[l] + bs[l]) + x
    return x
```

```python
import functools
import jax
import jax.numpy as jnp
import jax.experimental.pallas as pl
import jax.experimental.pallas.tpu as pltpu

f32 = jnp.float32
bf16 = jnp.bfloat16

A_ = {1: [(1,0),(1,3)], 2: [(1,2),(1,3)], 3: [(1,0)], 4: [(1,3)], 5: [(1,0),(1,1)], 6: [(1,2),(-1,0)], 7: [(1,1),(-1,3)]}
B_ = {1: [(1,0),(1,3)], 2: [(1,0)], 3: [(1,1),(-1,3)], 4: [(1,2),(-1,0)], 5: [(1,3)], 6: [(1,0),(1,1)], 7: [(1,2),(1,3)]}
C_ = {0: [(1,1),(1,4),(-1,5),(1,7)], 1: [(1,3),(1,5)], 2: [(1,2),(1,4)], 3: [(1,1),(-1,2),(1,3),(1,6)]}

def scheme(order, swapn):
    sw = (lambda j: j ^ 1) if swapn else (lambda j: j)
    prods = []
    for p in order:
        a = A_[p]
        b = [(s, sw(i)) for s, i in B_[p]]
        c = [(s, sw(ci)) for ci, terms in C_.items() for s, q in terms if q == p]
        prods.append((a, b, c))
    return prods

def lin(terms, blocks):
    terms = sorted(terms, key=lambda t: -t[0])
    acc = None
    for s, i in terms:
        if acc is None:
            acc = blocks[i] if s > 0 else -blocks[i]
        else:
            acc = acc + blocks[i] if s > 0 else acc - blocks[i]
    return acc

def ssum(terms):
    first = next(i for i, t in enumerate(terms) if t[0] > 0)
    acc = terms[first][1]()
    for i, (s_, m_) in enumerate(terms):
        if i == first: continue
        acc = acc + m_() if s_ > 0 else acc - m_()
    return acc

def make(bm=256, o1=(3,5,4,2,1,7,6), sw1=True, o2=(3,5,4,2,1,7,6), sw2=True, flags=None, prep=True, dyn='0xsmn', mpar=7, spar=7, PS=16):
    s1 = scheme(o1, sw1)
    s2 = scheme(o2, sw2)
    Q = 256
    R = bm // 4
    def last(s):
        return {k: max(p for p, (_, _, c) in enumerate(s) if any(i == k for _, i in c)) for k in range(4)}
    l1, l2 = last(s1), last(s2)
    def needs_store(s, lst, p):
        return any(lst[k] != p for _, k in s[p][2])

    def rs(k1, k2, R=R):
        r = (k1 // 2) * 2 + (k2 // 2); c = (k1 % 2) * 2 + (k2 % 2)
        return slice(r * R, (r + 1) * R), slice(c * Q, (c + 1) * Q)

    names = []
    K4 = [(a, b) for a in range(4) for b in range(4)]
    if '0' in dyn: names += [('0', k) for k in K4]
    if 'x' in dyn: names += [('x', (j, k)) for j in range(2) for k in K4]
    if 's' in dyn: names += [('s', (j, k)) for j in range(spar) for k in range(4)]
    if 'm' in dyn: names += [('m', (j, q)) for j in range(mpar) for q in range(7) if needs_store(s2, l2, q)]
    if 'n' in dyn: names += [('n', (p, k)) for p in range(7) for k in range(4) if needs_store(s1, l1, p)]

    def kern(x0_ref, w_hbm, b_ref, o_ref, wt_ref, w_ref, sem, *scr):
        L = w_ref.shape[0]
        @pl.when(pl.program_id(0) == 0)
        def _():
            for l in range(L):
                pltpu.make_async_copy(w_hbm.at[l], w_ref.at[l], sem.at[l]).start()
            def layer(l, _):
                pltpu.make_async_copy(w_hbm.at[l], w_ref.at[l], sem.at[l]).wait()
                def strip(j, _):
                    r0 = pl.multiple_of(j * PS, PS)
                    h0 = pl.multiple_of(j * (PS // 2), PS // 2)
                    def wblk(k1, k2):
                        r, c = rs(k1, k2, Q)
                        return w_ref[l, pl.ds(r.start + r0, PS), c].astype(f32)
                    for p, (_, b, _) in enumerate(s1):
                        tq = [lin(b, {k1: wblk(k1, k2) for _, k1 in b}) for k2 in range(4)]
                        for q, (_, b2, _) in enumerate(s2):
                            t = lin(b2, tq).astype(bf16)
                            wt_ref[l, p * 7 + q, pl.ds(h0, PS // 2), :] = pltpu.bitcast(t, jnp.int32)
                    return 0
                jax.lax.fori_loop(0, Q // PS, strip, 0)
                return 0
            jax.lax.fori_loop(0, L, layer, 0)
        z = pl.program_id(0) >> 20
        refs = dict(zip(names, scr))
        vals = {}
        def put(kind, key, v):
            if kind in dyn:
                refs[(kind, key)][0] = v
            else:
                vals[(kind, key)] = v
        def get(kind, key):
            if kind in dyn:
                return refs[(kind, key)][z]
            return vals[(kind, key)]
        done0 = set()
        def getx0(k):
            if k not in done0:
                done0.add(k)
                put('0', k, x0_ref[rs(*k)].astype(f32))
            return get('0', k)
        for l in range(L):
            getx = getx0 if l == 0 else (lambda k, l=l: get('x', (l % 2, k)))
            for p, (a, _, c) in enumerate(s1):
                sdone = set()
                def gets(k2):
                    if len(a) == 1:
                        return getx((a[0][1], k2))
                    if k2 not in sdone:
                        sdone.add(k2)
                        put('s', (p % spar, k2), lin(a, {k1: getx((k1, k2)) for _, k1 in a}))
                    return get('s', (p % spar, k2))
                for q, (a2, _, c2) in enumerate(s2):
                    w = pltpu.bitcast(wt_ref[l, p * 7 + q], bf16)
                    lhs = lin(a2, {k2: gets(k2) for _, k2 in a2}).astype(bf16)
                    m = jnp.dot(lhs, w, preferred_element_type=f32)
                    if needs_store(s2, l2, q):
                        put('m', (p % mpar, q), m)
                    for s, k2 in c2:
                        if l2[k2] != q: continue
                        terms = [(s_, (lambda q_=q_: m if q_ == q else get('m', (p % mpar, q_)))) for q_, (_, _, cc) in enumerate(s2) for s_, i in cc if i == k2]
                        c2v = ssum(terms)
                        if needs_store(s1, l1, p):
                            put('n', (p, k2), c2v)
                        for s_, k1 in c:
                            if l1[k1] != p: continue
                            terms1 = [(s__, (lambda p_=p_: c2v if p_ == p else get('n', (p_, k2)))) for p_, (_, _, cc) in enumerate(s1) for s__, i in cc if i == k1]
                            k = (k1, k2)
                            cv = ssum(terms1)
                            v = getx0(k) * (cv + b_ref[l:l+1, rs(*k)[1]].astype(f32)) + getx(k)
                            if l == L - 1:
                                o_ref[rs(*k)] = v.astype(bf16)
                            else:
                                put('x', ((l + 1) % 2, k), v)

    @jax.jit
    def f(x0, ws, bs):
        B, D = x0.shape
        L = ws.shape[0]

        return pl.pallas_call(
            kern,
            grid=(B // bm,),
            in_specs=[
                pl.BlockSpec((bm, D), lambda i: (i, 0)),
                pl.BlockSpec(memory_space=pl.ANY),
                pl.BlockSpec((L, D), lambda i: (0, 0), pipeline_mode=pl.Buffered(1)),
            ],
            out_specs=pl.BlockSpec((bm, D), lambda i: (i, 0)),
            out_shape=jax.ShapeDtypeStruct((B, D), x0.dtype),
            scratch_shapes=[pltpu.VMEM((L, 49, Q // 2, Q), jnp.int32), pltpu.VMEM((L, D, D), bf16), pltpu.SemaphoreType.DMA((L,))] + [pltpu.VMEM((1, R, Q), f32) for _ in names],
            compiler_params=pltpu.CompilerParams(
                dimension_semantics=("arbitrary",),
                vmem_limit_bytes=110 * 1024 * 1024,
                flags=flags,
            ),
        )(x0, ws, bs)
    return f


_impl = make()


@jax.jit
def pallas_standalone__dcn_v2_cross__recsys_kernel(x0: jax.Array, ws: jax.Array, bs: jax.Array):
    return _impl(x0, ws, bs)
```
